```python
import os as _os
_os.environ.setdefault("JAX_PLATFORMS", "cpu")
import jax
import jax.numpy as jnp

def _softmax(x, axis=-1):
    return jax.nn.softmax(x, axis=axis)
def _gelu(x):
    return jax.nn.gelu(x, approximate=True)
def _silu(x):
    return jax.nn.silu(x)
def _sigmoid(x):
    return jax.nn.sigmoid(x)
def _layernorm(x, axis=-1, eps=1e-5):
    m = jnp.mean(x, axis=axis, keepdims=True)
    v = jnp.var(x, axis=axis, keepdims=True)
    return (x - m) / jnp.sqrt(v + eps)
def _scatter_add(tgt, idx, src, axis=0):
    return tgt.at[idx].add(src)
def _segment_sum(src, seg, n):
    return jax.ops.segment_sum(src, seg, n)
class _Rng:
    def __init__(self, key):
        self._k = key
    def _next(self):
        self._k, sub = jax.random.split(self._k)
        return sub
    def normal(self, shape):
        return jax.random.normal(self._next(), shape, dtype=jnp.bfloat16)
    def randint(self, lo, hi, shape):
        return jax.random.randint(self._next(), shape, lo, hi, dtype=jnp.int32)
    def uniform(self, shape, lo=0.0, hi=1.0):
        return jax.random.uniform(self._next(), shape, jnp.bfloat16, lo, hi)
    def permutation(self, n):
        return jax.random.permutation(self._next(), n)


kernel_name = 'standalone__dcn_v2_cross__recsys'

def setup_inputs():
    _rng = _Rng(jax.random.key(int.from_bytes(__import__("os").urandom(4), "little")))
    _w = (lambda a: (lambda t: t.astype(jnp.bfloat16) if jnp.issubdtype(t.dtype, jnp.floating) else t)(jnp.asarray(a)))
    B, F, D, L = 4096, 26, 128, 6
    Din = min(F * D, 1024)
    return {
        "x0": _w((lambda *s: _rng.normal(s) * 0.05)(B, Din)),
        "ws": _w((lambda *s: _rng.normal(s) * 0.05)(L, Din, Din)),
        "bs": _w((lambda *s: _rng.normal(s) * 0.05)(L, Din)),
    }

def reference(x0, ws, bs):
    x = x0
    for l in range(ws.shape[0]):
        x = x0 * (x @ ws[l] + bs[l]) + x
    return x
```

```python
import functools

import jax
import jax.numpy as jnp
import jax.experimental.pallas as pl
import jax.experimental.pallas.tpu as pltpu


def _kernel(x0_ref, w_ref, b_ref, o_ref, x_ref, *, n_layers):
    l = pl.program_id(1)

    @pl.when(l == 0)
    def _():
        x_ref[...] = x0_ref[...]

    x = x_ref[...]
    acc = jnp.dot(x, w_ref[0], preferred_element_type=jnp.float32)
    y = x0_ref[...].astype(jnp.float32) * (acc + b_ref[0].astype(jnp.float32)) + x.astype(jnp.float32)
    y = y.astype(x_ref.dtype)
    x_ref[...] = y

    @pl.when(l == n_layers - 1)
    def _():
        o_ref[...] = y


@jax.jit
def pallas_standalone__dcn_v2_cross__recsys_kernel(
    x0: jax.Array,
    ws: jax.Array,
    bs: jax.Array,
):
    B, D = x0.shape
    L = ws.shape[0]
    tm = 1024
    bs3 = bs.reshape(L, 1, D)
    return pl.pallas_call(
        functools.partial(_kernel, n_layers=L),
        grid=(B // tm, L),
        in_specs=[
            pl.BlockSpec((tm, D), lambda i, l: (i, 0)),
            pl.BlockSpec((1, D, D), lambda i, l: (l, 0, 0)),
            pl.BlockSpec((1, 1, D), lambda i, l: (l, 0, 0)),
        ],
        out_specs=pl.BlockSpec((tm, D), lambda i, l: (i, 0)),
        out_shape=jax.ShapeDtypeStruct((B, D), x0.dtype),
        scratch_shapes=[pltpu.VMEM((tm, D), x0.dtype)],
        compiler_params=pltpu.CompilerParams(
            dimension_semantics=("parallel", "arbitrary"),
            vmem_limit_bytes=100 * 1024 * 1024,
        ),
    )(x0, ws, bs3)
```

```python
import functools
import jax
import jax.numpy as jnp
import jax.experimental.pallas as pl
import jax.experimental.pallas.tpu as pltpu

F32 = jnp.float32
BF16 = jnp.bfloat16


def _kernel(x0_hbm, w_hbm, b_hbm, o_hbm,
            x0_v, w_v, b_v, b32_v, o_v, acc_v,
            ksem, wsem, xsem, osem, *, L, D, R, tm, n, KC, NC):
    NKC = D // KC
    CW = D // NC

    def xk_copy(kc):
        k0 = kc * KC if isinstance(kc, int) else pl.multiple_of(kc * KC, KC)
        return pltpu.make_async_copy(x0_hbm.at[pl.ds(0, R), pl.ds(k0, KC)],
                                     x0_v.at[pl.ds(0, R), pl.ds(k0, KC)], ksem.at[kc])

    def wk_copy(kc):
        k0 = kc * KC if isinstance(kc, int) else pl.multiple_of(kc * KC, KC)
        return pltpu.make_async_copy(w_hbm.at[0, pl.ds(k0, KC), :],
                                     w_v.at[0, pl.ds(k0, KC), :], ksem.at[kc])

    b_copy = pltpu.make_async_copy(b_hbm, b_v, ksem.at[NKC - 1])

    def w_copy(l):
        return pltpu.make_async_copy(w_hbm.at[l], w_v.at[l], wsem.at[l - 1])

    def x_copy(i):
        r0 = R + i * tm
        if not isinstance(r0, int):
            r0 = pl.multiple_of(r0, 16)
        return pltpu.make_async_copy(x0_hbm.at[pl.ds(r0, tm)], x0_v.at[pl.ds(r0, tm)], xsem.at[i])

    def issue_k(kc, c):
        xk_copy(kc).start()
        wk_copy(kc).start()
        return c
    jax.lax.fori_loop(0, NKC, issue_k, 0)
    b_copy.start()

    def issue_w(l, c):
        w_copy(l).start()
        return c
    jax.lax.fori_loop(1, L, issue_w, 0)

    def issue_x(i, c):
        x_copy(i).start()
        return c
    jax.lax.fori_loop(0, n, issue_x, 0)

    acc_v[...] = jnp.zeros_like(acc_v)

    def kchunk(kc, c):
        k0 = pl.multiple_of(kc * KC, KC)
        xk_copy(kc).wait()
        wk_copy(kc).wait()
        acc_v[...] += jnp.dot(x0_v[pl.ds(0, R), pl.ds(k0, KC)], w_v[0, pl.ds(k0, KC), :],
                              preferred_element_type=F32)
        return c
    jax.lax.fori_loop(0, NKC - 1, kchunk, 0)
    kc = NKC - 1
    xk_copy(kc).wait()
    wk_copy(kc).wait()
    b_copy.wait()
    for l in range(L):
        b32_v[l] = b_v[l:l + 1, :].astype(F32)
    acc = acc_v[...] + jnp.dot(x0_v[pl.ds(0, R), pl.ds(kc * KC, KC)], w_v[0, pl.ds(kc * KC, KC), :],
                               preferred_element_type=F32)
    x0 = x0_v[pl.ds(0, R), :].astype(F32)
    o_v[pl.ds(0, R), :] = (x0 * (acc + b_v[0:1, :].astype(F32)) + x0).astype(BF16)

    def layer(l, c):
        w_copy(l).wait()
        xb = o_v[pl.ds(0, R), :]
        acc = jnp.dot(xb, w_v[l], preferred_element_type=F32)
        y = x0_v[pl.ds(0, R), :].astype(F32) * (acc + b32_v[l]) + xb.astype(F32)
        o_v[pl.ds(0, R), :] = y.astype(BF16)
        return c
    jax.lax.fori_loop(1, L, layer, 0)
    pltpu.make_async_copy(o_v.at[pl.ds(0, R)], o_hbm.at[pl.ds(0, R)], osem).start()

    def body(i, c):
        r0 = pl.multiple_of(R + i * tm, 16)
        x_copy(i).wait()
        x0b = x0_v[pl.ds(r0, tm), :]
        x0 = x0b.astype(F32)
        xb = x0b
        x = x0
        for l in range(L - 1):
            acc = jnp.dot(xb, w_v[l], preferred_element_type=F32)
            y = x0 * (acc + b32_v[l]) + x
            xb = y.astype(BF16)
            x = xb.astype(F32)
        l = L - 1
        for cc in range(NC):
            cs = slice(cc * CW, (cc + 1) * CW)
            acc = jnp.dot(xb, w_v[l, :, cs], preferred_element_type=F32)
            y = x0[:, cs] * (acc + b32_v[l, :, cs]) + x[:, cs]
            o_v[pl.ds(r0, tm), cs] = y.astype(BF16)
            pltpu.make_async_copy(o_v.at[pl.ds(r0, tm), pl.ds(cc * CW, CW)],
                                  o_hbm.at[pl.ds(r0, tm), pl.ds(cc * CW, CW)], osem).start()
        return c
    jax.lax.fori_loop(0, n, body, 0)
    pltpu.make_async_copy(o_v, o_hbm, osem).wait()


@jax.jit
def pallas_standalone__dcn_v2_cross__recsys_kernel(
    x0: jax.Array,
    ws: jax.Array,
    bs: jax.Array,
):
    B, D = x0.shape
    L = ws.shape[0]
    R, tm, KC, NC = 640, 576, 256, 8
    n = (B - R) // tm
    assert R + n * tm == B
    return pl.pallas_call(
        functools.partial(_kernel, L=L, D=D, R=R, tm=tm, n=n, KC=KC, NC=NC),
        in_specs=[
            pl.BlockSpec(memory_space=pl.ANY),
            pl.BlockSpec(memory_space=pl.ANY),
            pl.BlockSpec(memory_space=pl.ANY),
        ],
        out_specs=pl.BlockSpec(memory_space=pl.ANY),
        out_shape=jax.ShapeDtypeStruct((B, D), x0.dtype),
        scratch_shapes=[
            pltpu.VMEM((B, D), BF16),
            pltpu.VMEM((L, D, D), BF16),
            pltpu.VMEM((L, D), BF16),
            pltpu.VMEM((L, 1, D), F32),
            pltpu.VMEM((B, D), BF16),
            pltpu.VMEM((R, D), F32),
            pltpu.SemaphoreType.DMA((D // KC,)),
            pltpu.SemaphoreType.DMA((L - 1,)),
            pltpu.SemaphoreType.DMA((n,)),
            pltpu.SemaphoreType.DMA(()),
        ],
        compiler_params=pltpu.CompilerParams(
            vmem_limit_bytes=110 * 1024 * 1024,
        ),
    )(x0, ws, bs)
```

```python
import functools

import jax
import jax.numpy as jnp
import jax.experimental.pallas as pl
import jax.experimental.pallas.tpu as pltpu

F32 = jnp.float32
BF16 = jnp.bfloat16
LANE = 128
ROWS = 16


def _runs(chunks):
    out = []
    k = 0
    for i, s in enumerate(chunks):
        if out and out[-1][2] == s:
            out[-1][3] += 1
        else:
            out.append([i, k, s, 1])
        k += s
    return [tuple(g) for g in out]


def _halves(rows):
    lo = (rows // ROWS // 2) * ROWS
    return [rows - lo, lo]


def _dot(a, b):
    return jnp.dot(a, b, preferred_element_type=F32)


def _kernel(x0_hbm, w_hbm, b_hbm, o_hbm,
            x0_v, w_v, w0_v, b_v, b32_v, x1_v, o_v, acc_v,
            ksem, wsem, xsem, osem, *, L, D, R0, PR, Q, N, chunks):
    NT = D // LANE
    NK = len(chunks)
    P = N * PR

    def xk_copy(ci, k0, kc):
        return pltpu.make_async_copy(x0_hbm.at[pl.ds(0, R0), pl.ds(k0, kc)],
                                     x0_v.at[pl.ds(0, R0), pl.ds(k0, kc)], ksem.at[ci])

    def wk_copy(ci, k0, kc):
        return pltpu.make_async_copy(w_hbm.at[0, pl.ds(k0, kc), :],
                                     w0_v.at[pl.ds(k0, kc), :], ksem.at[ci])

    b_copy = pltpu.make_async_copy(b_hbm, b_v, ksem.at[NK - 1])
    bulk_copy = pltpu.make_async_copy(x0_hbm.at[pl.ds(R0, P - R0)],
                                      x0_v.at[pl.ds(R0, P - R0)], ksem.at[NK])

    def x_copy(i):
        r0 = pl.multiple_of(P + i * Q, ROWS)
        return pltpu.make_async_copy(x0_hbm.at[pl.ds(r0, Q)], x0_v.at[pl.ds(r0, Q)], xsem.at[i])

    def for_chunks(runs, fn):
        for c0, k0, kc, cnt in runs:
            def step(t, carry, c0=c0, k0=k0, kc=kc):
                fn(c0 + t, pl.multiple_of(k0 + t * kc, LANE), kc)
                return carry
            jax.lax.fori_loop(0, cnt, step, 0)

    def mm(xb, l, tiles=None):
        tiles = range(NT) if tiles is None else tiles
        if l == 0:
            return jnp.concatenate(
                [_dot(xb, w0_v[:, j * LANE:(j + 1) * LANE]) for j in tiles], axis=1)
        return jnp.concatenate([_dot(xb, w_v[l - 1, j]) for j in tiles], axis=1)

    def chunk_dot(k0, kc):
        return _dot(x0_v[pl.ds(0, R0), pl.ds(k0, kc)], w0_v[pl.ds(k0, kc), :])

    def issue_chunk(ci, k0, kc):
        xk_copy(ci, k0, kc).start()
        wk_copy(ci, k0, kc).start()
    for_chunks(_runs(chunks), issue_chunk)
    b_copy.start()
    bulk_copy.start()

    def issue_w(l, carry):
        for j in range(NT):
            pltpu.make_async_copy(w_hbm.at[l, :, pl.ds(j * LANE, LANE)],
                                  w_v.at[l - 1, j], wsem).start()
        return carry
    jax.lax.fori_loop(1, L, issue_w, 0)

    def issue_x(i, carry):
        x_copy(i).start()
        return carry
    jax.lax.fori_loop(0, N, issue_x, 0)

    def prologue():
        zr = 64

        def zero(t, carry):
            acc_v[pl.ds(pl.multiple_of(t * zr, zr), zr), :] = jnp.zeros((zr, D), F32)
            return carry
        jax.lax.fori_loop(0, R0 // zr, zero, 0)

        def accumulate(ci, k0, kc):
            xk_copy(ci, k0, kc).wait()
            wk_copy(ci, k0, kc).wait()
            acc_v[...] += chunk_dot(k0, kc)
        for_chunks(_runs(chunks[:-1]), accumulate)

        kc = chunks[-1]
        k0 = D - kc
        xk_copy(NK - 1, k0, kc).wait()
        wk_copy(NK - 1, k0, kc).wait()
        b_copy.wait()
        bulk_copy.wait()
        for l in range(L):
            b32_v[l] = b_v[l:l + 1, :].astype(F32)
        b0 = b_v[0:1, :].astype(F32)
        acc = acc_v[...] + chunk_dot(k0, kc)
        x0 = x0_v[pl.ds(0, R0), :].astype(F32)
        x1_v[pl.ds(0, R0), :] = (x0 * (acc + b0) + x0).astype(BF16)
        x0b = x0_v[pl.ds(R0, P - R0), :]
        x0 = x0b.astype(F32)
        x1_v[pl.ds(R0, P - R0), :] = (x0 * (mm(x0b, 0) + b0) + x0).astype(BF16)
        pltpu.make_async_copy(w_v, w_v, wsem).wait()

    def tile(i):
        a0 = pl.multiple_of(i * PR, ROWS)
        f0 = pl.multiple_of(P + i * Q, ROWS)
        x_copy(i).wait()
        x1p = x1_v[pl.ds(a0, PR), :]
        x0fb = x0_v[pl.ds(f0, Q), :]
        x0f = x0fb.astype(F32)
        x0 = jnp.concatenate([x0_v[pl.ds(a0, PR), :].astype(F32), x0f], axis=0)
        accp = mm(x1p, 1)
        x1f = (x0f * (mm(x0fb, 0) + b32_v[0]) + x0f).astype(BF16)
        acc = jnp.concatenate([accp, mm(x1f, 1)], axis=0)
        xb = jnp.concatenate([x1p, x1f], axis=0)
        x = xb.astype(F32)
        for l in range(1, L - 1):
            if l > 1:
                acc = mm(xb, l)
            xb = (x0 * (acc + b32_v[l]) + x).astype(BF16)
            x = xb.astype(F32)
        l = L - 1
        for j in range(NT):
            cs = slice(j * LANE, (j + 1) * LANE)
            yb = (x0[:, cs] * (mm(xb, l, [j]) + b32_v[l, :, cs]) + x[:, cs]).astype(BF16)
            last = j == NT - 1
            r = 0
            for base, rows in ((a0, PR), (f0, Q)):
                off = 0
                for s in (_halves(rows) if last else [rows]):
                    g = pl.multiple_of(base + off, ROWS)
                    o_v[pl.ds(g, s), cs] = yb[r:r + s]
                    pltpu.make_async_copy(o_v.at[pl.ds(g, s), pl.ds(j * LANE, LANE)],
                                          o_hbm.at[pl.ds(g, s), pl.ds(j * LANE, LANE)],
                                          osem).start()
                    off += s
                    r += s

    def step(i, carry):
        @pl.when(i == 0)
        def _():
            prologue()
        tile(i)
        return carry
    jax.lax.fori_loop(0, N, step, 0)
    pltpu.make_async_copy(o_v, o_hbm, osem).wait()


@jax.jit
def pallas_standalone__dcn_v2_cross__recsys_kernel(
    x0: jax.Array,
    ws: jax.Array,
    bs: jax.Array,
):
    B, D = x0.shape
    L = ws.shape[0]
    N, Q, R0 = 8, 224, 1024
    chunks = tuple(c * LANE for c in (1, 1, 2, 2, 2))
    PR = B // N - Q
    P = N * PR
    assert B % N == 0 and sum(chunks) == D and L >= 3
    assert PR % ROWS == 0 and Q % ROWS == 0 and R0 % 64 == 0 and R0 < P
    return pl.pallas_call(
        functools.partial(_kernel, L=L, D=D, R0=R0, PR=PR, Q=Q, N=N, chunks=chunks),
        in_specs=[
            pl.BlockSpec(memory_space=pl.ANY),
            pl.BlockSpec(memory_space=pl.ANY),
            pl.BlockSpec(memory_space=pl.ANY),
        ],
        out_specs=pl.BlockSpec(memory_space=pl.ANY),
        out_shape=jax.ShapeDtypeStruct((B, D), x0.dtype),
        scratch_shapes=[
            pltpu.VMEM((B, D), BF16),
            pltpu.VMEM((L - 1, D // LANE, D, LANE), BF16),
            pltpu.VMEM((D, D), BF16),
            pltpu.VMEM((L, D), BF16),
            pltpu.VMEM((L, 1, D), F32),
            pltpu.VMEM((P, D), BF16),
            pltpu.VMEM((B, D), BF16),
            pltpu.VMEM((R0, D), F32),
            pltpu.SemaphoreType.DMA((len(chunks) + 1,)),
            pltpu.SemaphoreType.DMA(()),
            pltpu.SemaphoreType.DMA((N,)),
            pltpu.SemaphoreType.DMA(()),
        ],
        compiler_params=pltpu.CompilerParams(
            vmem_limit_bytes=110 * 1024 * 1024,
            disable_bounds_checks=True,
            disable_semaphore_checks=True,
        ),
    )(x0, ws, bs)
```

```python
import functools

import jax
import jax.numpy as jnp
import jax.experimental.pallas as pl
import jax.experimental.pallas.tpu as pltpu

F32 = jnp.float32
BF16 = jnp.bfloat16
LANE = 128
ROWS = 16


def _runs(chunks, lo, hi):
    out = []
    k = sum(chunks[:lo])
    for i in range(lo, hi):
        s = chunks[i]
        if out and out[-1][2] == s:
            out[-1][3] += 1
        else:
            out.append([i, k, s, 1])
        k += s
    return [tuple(g) for g in out]


def _halves(rows):
    lo = (rows // ROWS // 2) * ROWS
    return [rows - lo, lo]


def _dot(a, b):
    return jnp.dot(a, b, preferred_element_type=F32)


def _kernel(x0_hbm, w_hbm, b_hbm, o_hbm,
            x0_v, w_v, w0_v, b_v, b32_v, x1_v, o_v, acc_v,
            ksem, wsem, xsem, osem, *, L, D, R0, RA, CA, PR, Q, N, chunks):
    NT = D // LANE
    NK = len(chunks)
    K0 = chunks[0]
    P = N * PR

    def xk_copy(ci, k0, kc):
        return pltpu.make_async_copy(x0_hbm.at[pl.ds(0, R0), pl.ds(k0, kc)],
                                     x0_v.at[pl.ds(0, R0), pl.ds(k0, kc)], ksem.at[ci])

    def wk_copy(ci, k0, kc):
        return pltpu.make_async_copy(w_hbm.at[0, pl.ds(k0, kc), :],
                                     w0_v.at[pl.ds(k0, kc), :], ksem.at[ci])

    def x0_piece(r0, rows, sem):
        return pltpu.make_async_copy(x0_hbm.at[pl.ds(r0, rows), pl.ds(0, K0)],
                                     x0_v.at[pl.ds(r0, rows), pl.ds(0, K0)], sem)

    def w0_piece(c0, cols, sem):
        return pltpu.make_async_copy(w_hbm.at[0, pl.ds(0, K0), pl.ds(c0, cols)],
                                     w0_v.at[pl.ds(0, K0), pl.ds(c0, cols)], sem)

    corner = (x0_piece(0, RA, ksem.at[NK + 1]), w0_piece(0, CA, ksem.at[NK + 1]))
    rest = (x0_piece(RA, R0 - RA, ksem.at[0]), w0_piece(CA, D - CA, ksem.at[0]))
    b_copy = pltpu.make_async_copy(b_hbm, b_v, ksem.at[NK - 1])
    bulk_copy = pltpu.make_async_copy(x0_hbm.at[pl.ds(R0, P - R0)],
                                      x0_v.at[pl.ds(R0, P - R0)], ksem.at[NK])

    def x_copy(i):
        r0 = pl.multiple_of(P + i * Q, ROWS)
        return pltpu.make_async_copy(x0_hbm.at[pl.ds(r0, Q)], x0_v.at[pl.ds(r0, Q)], xsem.at[i])

    def for_chunks(runs, fn):
        for c0, k0, kc, cnt in runs:
            def step(t, carry, c0=c0, k0=k0, kc=kc):
                fn(c0 + t, pl.multiple_of(k0 + t * kc, LANE), kc)
                return carry
            jax.lax.fori_loop(0, cnt, step, 0)

    def mm(xb, l, tiles=None):
        tiles = range(NT) if tiles is None else tiles
        if l == 0:
            return jnp.concatenate(
                [_dot(xb, w0_v[:, j * LANE:(j + 1) * LANE]) for j in tiles], axis=1)
        return jnp.concatenate([_dot(xb, w_v[l - 1, j]) for j in tiles], axis=1)

    def chunk_dot(k0, kc):
        return _dot(x0_v[pl.ds(0, R0), pl.ds(k0, kc)], w0_v[pl.ds(k0, kc), :])

    def issue_first(t, carry):
        @pl.when(t == 0)
        def _():
            for c in corner:
                c.start()

        @pl.when(t == 1)
        def _():
            for c in rest:
                c.start()
        return carry
    jax.lax.fori_loop(0, 2, issue_first, 0)

    def issue_chunk(ci, k0, kc):
        xk_copy(ci, k0, kc).start()
        wk_copy(ci, k0, kc).start()
    for_chunks(_runs(chunks, 1, NK), issue_chunk)
    b_copy.start()
    bulk_copy.start()

    def issue_w(l, carry):
        for j in range(NT):
            pltpu.make_async_copy(w_hbm.at[l, :, pl.ds(j * LANE, LANE)],
                                  w_v.at[l - 1, j], wsem).start()
        return carry
    jax.lax.fori_loop(1, L, issue_w, 0)

    def issue_x(i, carry):
        x_copy(i).start()
        return carry
    jax.lax.fori_loop(0, N, issue_x, 0)

    def prologue():
        def first_dot(r0, rows, c0, cols):
            acc_v[pl.ds(r0, rows), pl.ds(c0, cols)] = _dot(
                x0_v[pl.ds(r0, rows), pl.ds(0, K0)], w0_v[pl.ds(0, K0), pl.ds(c0, cols)])

        for c in corner:
            c.wait()
        first_dot(0, RA, 0, CA)
        for c in rest:
            c.wait()
        first_dot(0, RA, CA, D - CA)
        first_dot(RA, R0 - RA, 0, D)

        def accumulate(ci, k0, kc):
            xk_copy(ci, k0, kc).wait()
            wk_copy(ci, k0, kc).wait()
            acc_v[...] += chunk_dot(k0, kc)
        for_chunks(_runs(chunks, 1, NK - 1), accumulate)

        kc = chunks[-1]
        k0 = D - kc
        xk_copy(NK - 1, k0, kc).wait()
        wk_copy(NK - 1, k0, kc).wait()
        b_copy.wait()
        bulk_copy.wait()
        for l in range(L):
            b32_v[l] = b_v[l:l + 1, :].astype(F32)
        b0 = b_v[0:1, :].astype(F32)
        acc = acc_v[...] + chunk_dot(k0, kc)
        x0 = x0_v[pl.ds(0, R0), :].astype(F32)
        x1_v[pl.ds(0, R0), :] = (x0 * (acc + b0) + x0).astype(BF16)
        x0b = x0_v[pl.ds(R0, P - R0), :]
        x0 = x0b.astype(F32)
        x1_v[pl.ds(R0, P - R0), :] = (x0 * (mm(x0b, 0) + b0) + x0).astype(BF16)
        pltpu.make_async_copy(w_v, w_v, wsem).wait()

    def tile(i):
        a0 = pl.multiple_of(i * PR, ROWS)
        f0 = pl.multiple_of(P + i * Q, ROWS)
        x_copy(i).wait()
        x1p = x1_v[pl.ds(a0, PR), :]
        x0fb = x0_v[pl.ds(f0, Q), :]
        x0f = x0fb.astype(F32)
        x0 = jnp.concatenate([x0_v[pl.ds(a0, PR), :].astype(F32), x0f], axis=0)
        accp = mm(x1p, 1)
        x1f = (x0f * (mm(x0fb, 0) + b32_v[0]) + x0f).astype(BF16)
        acc = jnp.concatenate([accp, mm(x1f, 1)], axis=0)
        xb = jnp.concatenate([x1p, x1f], axis=0)
        x = xb.astype(F32)
        for l in range(1, L - 1):
            if l > 1:
                acc = mm(xb, l)
            xb = (x0 * (acc + b32_v[l]) + x).astype(BF16)
            x = xb.astype(F32)
        l = L - 1
        for j in range(NT):
            cs = slice(j * LANE, (j + 1) * LANE)
            yb = (x0[:, cs] * (mm(xb, l, [j]) + b32_v[l, :, cs]) + x[:, cs]).astype(BF16)
            last = j == NT - 1
            r = 0
            for base, rows in ((a0, PR), (f0, Q)):
                off = 0
                for s in (_halves(rows) if last else [rows]):
                    g = pl.multiple_of(base + off, ROWS)
                    o_v[pl.ds(g, s), cs] = yb[r:r + s]
                    pltpu.make_async_copy(o_v.at[pl.ds(g, s), pl.ds(j * LANE, LANE)],
                                          o_hbm.at[pl.ds(g, s), pl.ds(j * LANE, LANE)],
                                          osem).start()
                    off += s
                    r += s

    def step(i, carry):
        @pl.when(i == 0)
        def _():
            prologue()
        tile(i)
        return carry
    jax.lax.fori_loop(0, N, step, 0)
    pltpu.make_async_copy(o_v, o_hbm, osem).wait()


@jax.jit
def pallas_standalone__dcn_v2_cross__recsys_kernel(
    x0: jax.Array,
    ws: jax.Array,
    bs: jax.Array,
):
    B, D = x0.shape
    L = ws.shape[0]
    N, Q, R0, RA, CA = 8, 224, 1536, 512, 512
    chunks = tuple(c * LANE for c in (1, 2, 2, 3))
    PR = B // N - Q
    P = N * PR
    assert B % N == 0 and sum(chunks) == D and L >= 3
    assert PR % ROWS == 0 and Q % ROWS == 0 and RA < R0 < P and CA < D
    return pl.pallas_call(
        functools.partial(_kernel, L=L, D=D, R0=R0, RA=RA, CA=CA, PR=PR, Q=Q, N=N, chunks=chunks),
        in_specs=[
            pl.BlockSpec(memory_space=pl.ANY),
            pl.BlockSpec(memory_space=pl.ANY),
            pl.BlockSpec(memory_space=pl.ANY),
        ],
        out_specs=pl.BlockSpec(memory_space=pl.ANY),
        out_shape=jax.ShapeDtypeStruct((B, D), x0.dtype),
        scratch_shapes=[
            pltpu.VMEM((B, D), BF16),
            pltpu.VMEM((L - 1, D // LANE, D, LANE), BF16),
            pltpu.VMEM((D, D), BF16),
            pltpu.VMEM((L, D), BF16),
            pltpu.VMEM((L, 1, D), F32),
            pltpu.VMEM((P, D), BF16),
            pltpu.VMEM((B, D), BF16),
            pltpu.VMEM((R0, D), F32),
            pltpu.SemaphoreType.DMA((len(chunks) + 2,)),
            pltpu.SemaphoreType.DMA(()),
            pltpu.SemaphoreType.DMA((N,)),
            pltpu.SemaphoreType.DMA(()),
        ],
        compiler_params=pltpu.CompilerParams(
            vmem_limit_bytes=110 * 1024 * 1024,
            disable_bounds_checks=True,
            disable_semaphore_checks=True,
        ),
    )(x0, ws, bs)
```
